```python
import os as _os
_os.environ.setdefault("JAX_PLATFORMS", "cpu")
import jax
import jax.numpy as jnp

def _softmax(x, axis=-1):
    return jax.nn.softmax(x, axis=axis)
def _gelu(x):
    return jax.nn.gelu(x, approximate=True)
def _silu(x):
    return jax.nn.silu(x)
def _sigmoid(x):
    return jax.nn.sigmoid(x)
def _layernorm(x, axis=-1, eps=1e-5):
    m = jnp.mean(x, axis=axis, keepdims=True)
    v = jnp.var(x, axis=axis, keepdims=True)
    return (x - m) / jnp.sqrt(v + eps)
def _scatter_add(tgt, idx, src, axis=0):
    return tgt.at[idx].add(src)
def _segment_sum(src, seg, n):
    return jax.ops.segment_sum(src, seg, n)
class _Rng:
    def __init__(self, key):
        self._k = key
    def _next(self):
        self._k, sub = jax.random.split(self._k)
        return sub
    def normal(self, shape):
        return jax.random.normal(self._next(), shape, dtype=jnp.bfloat16)
    def randint(self, lo, hi, shape):
        return jax.random.randint(self._next(), shape, lo, hi, dtype=jnp.int32)
    def uniform(self, shape, lo=0.0, hi=1.0):
        return jax.random.uniform(self._next(), shape, jnp.bfloat16, lo, hi)
    def permutation(self, n):
        return jax.random.permutation(self._next(), n)


kernel_name = 'concat_heads__compressed_kv_cla__compressed_kv_cla__decode'

def setup_inputs():
    _rng = _Rng(jax.random.key(int.from_bytes(__import__("os").urandom(4), "little")))
    _w = (lambda a: (lambda t: t.astype(jnp.bfloat16) if jnp.issubdtype(t.dtype, jnp.floating) else t)(jnp.asarray(a)))
    def _A_setup():
        B, H, Sq, Sk, D, M = 4, 32, 1, 4096, 128, 640
        Dc = 4 * D
        return {
            "x": _w((lambda *s: _rng.normal(s) * 1.6)(B, Sq, M)),
            "c_kv": _w((lambda *s: _rng.normal(s) * 0.05)(B, Sk, Dc)),
            "w_q": _w((lambda *s: _rng.normal(s) * 1.6)(M, H, D) * (M ** -0.5)),
            "w_uk": _w((lambda *s: _rng.normal(s) * 1.6)(Dc, H, D) * (Dc ** -0.5)),
            "w_uv": _w((lambda *s: _rng.normal(s) * 0.05)(Dc, H, D) * (Dc ** -0.5)),
            "w_o": _w((lambda *s: _rng.normal(s) * 0.05)(H, D, M) * ((H * D) ** -0.5)),
        }
    _A_in = _A_setup()

    def _B_setup():
        B, H, Sq, Sk, D, M = 4, 32, 1, 4096, 128, 640
        Dc = 4 * D
        return {
            "x": _w((lambda *s: _rng.normal(s) * 1.6)(B, Sq, M)),
            "c_kv": _w((lambda *s: _rng.normal(s) * 0.05)(B, Sk, Dc)),
            "w_q": _w((lambda *s: _rng.normal(s) * 1.6)(M, H, D) * (M ** -0.5)),
            "w_uk": _w((lambda *s: _rng.normal(s) * 1.6)(Dc, H, D) * (Dc ** -0.5)),
            "w_uv": _w((lambda *s: _rng.normal(s) * 0.05)(Dc, H, D) * (Dc ** -0.5)),
            "w_o": _w((lambda *s: _rng.normal(s) * 0.05)(H, D, M) * ((H * D) ** -0.5)),
        }
    _B_in = _B_setup()

    return {
        "A_x": _A_in["x"],
        "A_c_kv": _A_in["c_kv"],
        "A_w_q": _A_in["w_q"],
        "A_w_uk": _A_in["w_uk"],
        "A_w_uv": _A_in["w_uv"],
        "A_w_o": _A_in["w_o"],
        "B_x": _B_in["x"],
        "B_c_kv": _B_in["c_kv"],
        "B_w_q": _B_in["w_q"],
        "B_w_uk": _B_in["w_uk"],
        "B_w_uv": _B_in["w_uv"],
        "B_w_o": _B_in["w_o"],
    }

def reference(A_x, A_c_kv, A_w_q, A_w_uk, A_w_uv, A_w_o, B_x, B_c_kv, B_w_q, B_w_uk, B_w_uv, B_w_o):
    def _A_ref(x, c_kv, w_q, w_uk, w_uv, w_o):
        B, Sq, M = x.shape[0], x.shape[1], x.shape[2]
        Sk = c_kv.shape[1]
        H, D = w_q.shape[1], w_q.shape[2]
        q = jnp.einsum("bqm,mhd->bhqd", x, w_q)
        k = jnp.einsum("bkc,chd->bhkd", c_kv, w_uk)
        v = jnp.einsum("bkc,chd->bhkd", c_kv, w_uv)
        scores = jnp.einsum("bhqd,bhkd->bhqk", q, k) * (D ** -0.5)
        off = Sk - Sq
        qi = jnp.arange(Sq)[:, None]
        kj = jnp.arange(Sk)[None, :]
        cmask = kj <= (qi + off)
        scores = jnp.where(cmask[None, None], scores, -1e9)
        p = _softmax(scores, axis=-1)
        ctx = jnp.einsum("bhqk,bhkd->bhqd", p, v)
        return jnp.einsum("bhqd,hdm->bqm", ctx, w_o)

    def _B_ref(x, c_kv, w_q, w_uk, w_uv, w_o):
        B, Sq, M = x.shape[0], x.shape[1], x.shape[2]
        Sk = c_kv.shape[1]
        H, D = w_q.shape[1], w_q.shape[2]
        q = jnp.einsum("bqm,mhd->bhqd", x, w_q)
        k = jnp.einsum("bkc,chd->bhkd", c_kv, w_uk)
        v = jnp.einsum("bkc,chd->bhkd", c_kv, w_uv)
        scores = jnp.einsum("bhqd,bhkd->bhqk", q, k) * (D ** -0.5)
        off = Sk - Sq
        qi = jnp.arange(Sq)[:, None]
        kj = jnp.arange(Sk)[None, :]
        cmask = kj <= (qi + off)
        scores = jnp.where(cmask[None, None], scores, -1e9)
        p = _softmax(scores, axis=-1)
        ctx = jnp.einsum("bhqk,bhkd->bhqd", p, v)
        return jnp.einsum("bhqd,hdm->bqm", ctx, w_o)

    a = _A_ref(A_x, A_c_kv, A_w_q, A_w_uk, A_w_uv, A_w_o)
    b = _B_ref(B_x, B_c_kv, B_w_q, B_w_uk, B_w_uv, B_w_o)
    return jnp.concatenate([a, b], axis=-1)
```

```python
import functools
import jax
import jax.numpy as jnp
from jax.experimental import pallas as pl
from jax.experimental.pallas import tpu as pltpu

B, H, SK, D, M = 4, 32, 4096, 128, 640
DC = 4 * D
NT = (((1,), (1,)), ((), ()))
NN = (((1,), (0,)), ((), ()))
F32 = jnp.float32
BF16 = jnp.bfloat16

WO_CHUNKS = ((16, 16), (12, 12, 4, 2, 1, 1))
NSEM = 4


def _dot(a, b, dims):
    return jax.lax.dot_general(a, b, dims, preferred_element_type=F32)


def _kernel(ax, ac, awq, awuk, awuv, awo, bx, bc, bwq, bwuk, bwuv, bwo,
            o_ref,
            x_s, c_s, wq_s, wuk_s, wuv_s, wo_s,
            e_s, xr_s, qat_s, qa_s, cc_s, ctx_s, sems):
    hbm = ((ax, ac, awq, awuk, awuv, awo), (bx, bc, bwq, bwuk, bwuv, bwo))

    groups = []
    for br in range(2):
        x, c, wq, wuk, wuv, wo = hbm[br]
        g0 = [(wq, wq_s.at[br])]
        if br == 0:
            g0 = [(ax, x_s.at[0]), (bx, x_s.at[1])] + g0
        groups.append(g0)
        groups.append([(wuk, wuk_s.at[br])])
        for b in range(B):
            groups.append([(c.at[b], c_s.at[br, b])])
        for t in range(4):
            groups.append([(wuv.at[pl.ds(128 * t, 128)], wuv_s.at[br, pl.ds(128 * t, 128)])])
        h0 = 0
        for n in WO_CHUNKS[br]:
            groups.append([(wo.at[pl.ds(h0, n)], wo_s.at[br, pl.ds(h0, n)])])
            h0 += n
    cps = [[pltpu.make_async_copy(s, d, sems.at[i % NSEM]) for (s, d) in g] for i, g in enumerate(groups)]
    state = {"next": 0}

    def start(i):
        if i < len(cps):
            for cp in cps[i]:
                cp.start()

    def acquire():
        i = state["next"]
        state["next"] = i + 1
        for cp in cps[i]:
            cp.wait()
        start(i + NSEM)

    for i in range(NSEM):
        start(i)

    r_io = jax.lax.broadcasted_iota(jnp.int32, (128, 2048), 0)
    l_io = jax.lax.broadcasted_iota(jnp.int32, (128, 2048), 1)
    e_s[...] = jnp.where(r_io == (l_io >> 4), 1.0, 0.0).astype(BF16)

    def branch(br):
        acquire()
        x = x_s[br].astype(F32)
        z4 = jnp.zeros((4, 128), F32)
        pieces = []
        for t in range(5):
            pieces += [x[:, 128 * t:128 * (t + 1)], z4]
        pieces.append(jnp.zeros((8, 128), F32))
        xs = jnp.concatenate(pieces, axis=0).astype(BF16)
        xr_s[...] = _dot(xs, e_s[...], NN)

        row = jax.lax.broadcasted_iota(jnp.int32, (64, 2048), 0)
        lane = jax.lax.broadcasted_iota(jnp.int32, (64, 2048), 1)
        m64 = (row & 15) == (lane & 15)

        def s1(t, acc):
            q0, q1 = acc
            rows = [jnp.broadcast_to(xr_s[pl.ds(8 * t + b, 1), :], (16, 2048)) for b in range(B)]
            lt = jnp.where(m64, jnp.concatenate(rows, axis=0), 0.0).astype(BF16)
            m0 = pl.multiple_of(128 * t, 128)
            w0 = wq_s[br, pl.ds(m0, 128), 0:16, :].reshape(2048, 128)
            w1 = wq_s[br, pl.ds(m0, 128), 16:32, :].reshape(2048, 128)
            return q0 + _dot(lt, w0, NN), q1 + _dot(lt, w1, NN)

        q0, q1 = jax.lax.fori_loop(0, 5, s1, (jnp.zeros((64, 128), F32), jnp.zeros((64, 128), F32)))
        qall = jnp.concatenate([q0, q1], axis=0).astype(BF16)

        acquire()
        CC = 32
        hh = jax.lax.broadcasted_iota(jnp.int32, (CC, 32, 128), 1)
        ll = jax.lax.broadcasted_iota(jnp.int32, (CC, 32, 128), 2)
        m2 = hh == ((ll >> 6) * 16 + (ll & 15))

        def s2(i, carry):
            c0 = pl.multiple_of(CC * i, CC)
            w = wuk_s[br, pl.ds(c0, CC), :, :].reshape(CC * 32, 128)
            r = _dot(w, qall, NT).reshape(CC, 32, 128)
            qat_s[pl.ds(c0, CC), :] = jnp.sum(jnp.where(m2, r, 0.0), axis=1)
            return carry

        jax.lax.fori_loop(0, DC // CC, s2, 0)
        qa_s[...] = (qat_s[...].T * (D ** -0.5)).astype(BF16)

        for b in range(B):
            acquire()
            qb = jnp.concatenate([qa_s[16 * b:16 * b + 16, :], qa_s[64 + 16 * b:64 + 16 * b + 16, :]], axis=0)
            s = _dot(qb, c_s[br, b], NT)
            m = jnp.max(s, axis=1, keepdims=True)
            p = jnp.exp(s - m)
            l = jnp.sum(p, axis=1, keepdims=True)
            cc = (_dot(p.astype(BF16), c_s[br, b], NN) / l).astype(BF16)
            for t in range(4):
                cc_s[t, 16 * b:16 * b + 16, :] = cc[0:16, 128 * t:128 * (t + 1)]
                cc_s[t, 64 + 16 * b:64 + 16 * b + 16, :] = cc[16:32, 128 * t:128 * (t + 1)]

        row = jax.lax.broadcasted_iota(jnp.int32, (128, 2048), 0)
        lane = jax.lax.broadcasted_iota(jnp.int32, (128, 2048), 1)
        m128 = (row & 15) == (lane & 15)
        c0acc = jnp.zeros((64, 128), F32)
        c1acc = jnp.zeros((64, 128), F32)
        for t in range(4):
            ex = jnp.where(m128, _dot(cc_s[t], e_s[...], NN), 0.0).astype(BF16)
            acquire()
            w0 = wuv_s[br, 128 * t:128 * (t + 1), 0:16, :].reshape(2048, 128)
            w1 = wuv_s[br, 128 * t:128 * (t + 1), 16:32, :].reshape(2048, 128)
            c0acc = c0acc + _dot(ex[0:64], w0, NN)
            c1acc = c1acc + _dot(ex[64:128], w1, NN)
        ctx_s[0] = c0acc.reshape(4, 16, 128)
        ctx_s[1] = c1acc.reshape(4, 16, 128)

        out = jnp.zeros((4, M), F32)
        h0 = 0
        for n in WO_CHUNKS[br]:
            lhs = jnp.concatenate([ctx_s[h // 16, :, h % 16, :] for h in range(h0, h0 + n)], axis=1).astype(BF16)
            acquire()
            out = out + _dot(lhs, wo_s[br, h0:h0 + n].reshape(n * 128, M), NN)
            h0 += n
        o_ref[:, M * br:M * (br + 1)] = out.astype(o_ref.dtype)

    branch(0)
    branch(1)
    assert state["next"] == len(cps)


@jax.jit
def pallas_concat_heads__compressed_kv_cla__compressed_kv_cla__decode_kernel(A_x, A_c_kv, A_w_q, A_w_uk, A_w_uv, A_w_o, B_x, B_c_kv, B_w_q, B_w_uk, B_w_uv, B_w_o):
    out = pl.pallas_call(
        _kernel,
        out_shape=jax.ShapeDtypeStruct((B, 2 * M), BF16),
        in_specs=[pl.BlockSpec(memory_space=pl.ANY)] * 12,
        scratch_shapes=[
            pltpu.VMEM((2, B, M), BF16),
            pltpu.VMEM((2, B, SK, DC), BF16),
            pltpu.VMEM((2, M, H, D), BF16),
            pltpu.VMEM((2, DC, H, D), BF16),
            pltpu.VMEM((2, DC, H, D), BF16),
            pltpu.VMEM((2, H, D, M), BF16),
            pltpu.VMEM((128, 2048), BF16),
            pltpu.VMEM((48, 2048), F32),
            pltpu.VMEM((DC, 128), F32),
            pltpu.VMEM((128, DC), BF16),
            pltpu.VMEM((4, 128, 128), BF16),
            pltpu.VMEM((2, 4, 16, 128), F32),
            pltpu.SemaphoreType.DMA((NSEM,)),
        ],
        compiler_params=pltpu.CompilerParams(vmem_limit_bytes=110 * 1024 * 1024),
    )(A_x.reshape(B, M), A_c_kv, A_w_q, A_w_uk, A_w_uv, A_w_o,
      B_x.reshape(B, M), B_c_kv, B_w_q, B_w_uk, B_w_uv, B_w_o)
    return out.reshape(B, 1, 2 * M)
```

```python
import jax
import jax.numpy as jnp
from jax.experimental import pallas as pl
from jax.experimental.pallas import tpu as pltpu

B, H, SK, D, M = 4, 32, 4096, 128, 640
DC = 4 * D
NN = (((1,), (0,)), ((), ()))
NT = (((1,), (1,)), ((), ()))
F32 = jnp.float32
BF16 = jnp.bfloat16

CHAIN_ROWS = (96, 80, 96, 80, 96, 80, 96, 128, 96, 80, 96, 80, 96, 80)
CHAIN_TOTAL = sum(CHAIN_ROWS)
WO_ROWS = ((2048, 2048), (1408, 1024, 256, 128))
assert CHAIN_TOTAL % D == 0 and CHAIN_TOTAL + sum(WO_ROWS[1]) == H * D == sum(WO_ROWS[0])
N_COPIES = 2 * (3 + B + 4) + len(WO_ROWS[0]) + len(WO_ROWS[1])
S2_ROWS = 32


def _dot(a, b, dims):
    return jax.lax.dot_general(a, b, dims, preferred_element_type=F32)


def _iota(shape, dim):
    return jax.lax.broadcasted_iota(jnp.int32, shape, dim)


def _kernel(ax, ac, awq, awuk, awuv, awo, bx, bc, bwq, bwuk, bwuv, bwo,
            o_ref,
            x_s, c_s, wq_s, wuk_s, wuv_s, wo_s, stage_s,
            e_s, xr_s, qat_s, qa_s, cc_s, ctx_s, lhs_s, sems, chain_sems):
    hbm = ((ax, ac, awq, awuk, awuv, awo), (bx, bc, bwq, bwuk, bwuv, bwo))

    copies, tick = [], []

    def add(src, dst, t=False):
        copies.append(pltpu.make_async_copy(src, dst, sems.at[len(copies)]))
        tick.append(t)

    for br in range(2):
        x, c, wq, wuk, wuv, wo = hbm[br]
        add(wq, wq_s.at[br])
        add(x, x_s.at[br], True)
        add(wuk, wuk_s.at[br], True)
        for b in range(B):
            add(c.at[b], c_s.at[br, b], True)
        for t in range(4):
            add(wuv.at[pl.ds(D * t, D)], wuv_s.at[br, pl.ds(D * t, D)], br == 0 and t == 3)
        r0 = 0 if br == 0 else CHAIN_TOTAL
        for k, n in enumerate(WO_ROWS[br]):
            add(wo.at[pl.ds(r0, n)], wo_s.at[br, pl.ds(r0, n)], br == 0 and k == len(WO_ROWS[0]) - 1)
            r0 += n
    assert len(copies) == N_COPIES

    nch = len(CHAIN_ROWS)
    assert sum(tick) == nch
    offs = [sum(CHAIN_ROWS[:j]) for j in range(nch)]
    h2s = [pltpu.make_async_copy(bwo.at[pl.ds(offs[j], r)], stage_s.at[j % 2, pl.ds(0, r)], chain_sems.at[0])
           for j, r in enumerate(CHAIN_ROWS)]
    s2v = [pltpu.make_async_copy(stage_s.at[j % 2, pl.ds(0, r)], wo_s.at[1, pl.ds(offs[j], r)], chain_sems.at[1])
           for j, r in enumerate(CHAIN_ROWS)]
    state = {"copy": 0, "chain": 0}

    def chain_step():
        j = state["chain"]
        state["chain"] = j + 1
        if j >= 1:
            s2v[j - 1].wait()
        if j < nch:
            h2s[j].wait()
            s2v[j].start(priority=1)
            if j + 1 < nch:
                h2s[j + 1].start(priority=1)

    def acquire():
        i = state["copy"]
        state["copy"] = i + 1
        copies[i].wait()
        if tick[i]:
            chain_step()

    copies[0].start()
    h2s[0].start(priority=1)
    for cp in copies[1:]:
        cp.start()

    e_s[...] = jnp.where(_iota((128, 2048), 0) == (_iota((128, 2048), 1) >> 4), 1.0, 0.0).astype(BF16)

    def branch(br):
        acquire()
        acquire()
        x = x_s[br].astype(F32)
        pieces = []
        for t in range(5):
            pieces += [x[:, 128 * t:128 * (t + 1)], jnp.zeros((4, 128), F32)]
        pieces.append(jnp.zeros((8, 128), F32))
        xs = jnp.concatenate(pieces, axis=0).astype(BF16)
        xr_s[...] = _dot(xs, e_s[...], NN)
        m64 = (_iota((64, 2048), 0) & 15) == (_iota((64, 2048), 1) & 15)

        def q_step(t, acc):
            q0, q1 = acc
            rows = [jnp.broadcast_to(xr_s[pl.ds(8 * t + b, 1), :], (16, 2048)) for b in range(B)]
            lt = jnp.where(m64, jnp.concatenate(rows, axis=0), 0.0).astype(BF16)
            m0 = pl.multiple_of(128 * t, 128)
            w0 = wq_s[br, pl.ds(m0, 128), 0:16, :].reshape(2048, D)
            w1 = wq_s[br, pl.ds(m0, 128), 16:32, :].reshape(2048, D)
            return q0 + _dot(lt, w0, NN), q1 + _dot(lt, w1, NN)

        zero = jnp.zeros((64, D), F32)
        q0, q1 = jax.lax.fori_loop(0, M // 128, q_step, (zero, zero))
        q_all = jnp.concatenate([q0, q1], axis=0).astype(BF16)

        acquire()
        lanes = _iota((S2_ROWS, H, 128), 2)
        m2 = _iota((S2_ROWS, H, 128), 1) == ((lanes >> 6) * 16 + (lanes & 15))

        def qa_step(i, carry):
            c0 = pl.multiple_of(S2_ROWS * i, S2_ROWS)
            w = wuk_s[br, pl.ds(c0, S2_ROWS), :, :].reshape(S2_ROWS * H, D)
            r = _dot(w, q_all, NT).reshape(S2_ROWS, H, 128)
            qat_s[pl.ds(c0, S2_ROWS), :] = jnp.sum(jnp.where(m2, r, 0.0), axis=1)
            return carry

        jax.lax.fori_loop(0, DC // S2_ROWS, qa_step, 0)
        qa_s[...] = (qat_s[...].T * (D ** -0.5)).astype(BF16)

        for b in range(B):
            acquire()
            qb = jnp.concatenate([qa_s[16 * b:16 * b + 16, :], qa_s[64 + 16 * b:64 + 16 * b + 16, :]], axis=0)
            s = _dot(qb, c_s[br, b], NT)
            p = jnp.exp(s - jnp.max(s, axis=1, keepdims=True))
            l = jnp.sum(p, axis=1, keepdims=True)
            cc = (_dot(p.astype(BF16), c_s[br, b], NN) / l).astype(BF16)
            for t in range(4):
                cc_s[t, 16 * b:16 * b + 16, :] = cc[0:16, 128 * t:128 * (t + 1)]
                cc_s[t, 64 + 16 * b:64 + 16 * b + 16, :] = cc[16:32, 128 * t:128 * (t + 1)]

        m128 = (_iota((128, 2048), 0) & 15) == (_iota((128, 2048), 1) & 15)
        ctx0 = jnp.zeros((64, D), F32)
        ctx1 = jnp.zeros((64, D), F32)
        for t in range(4):
            ex = jnp.where(m128, _dot(cc_s[t], e_s[...], NN), 0.0).astype(BF16)
            acquire()
            w0 = wuv_s[br, 128 * t:128 * (t + 1), 0:16, :].reshape(2048, D)
            w1 = wuv_s[br, 128 * t:128 * (t + 1), 16:32, :].reshape(2048, D)
            ctx0 = ctx0 + _dot(ex[0:64], w0, NN)
            ctx1 = ctx1 + _dot(ex[64:128], w1, NN)
        ctx_s[0] = ctx0.reshape(B, 16, D)
        ctx_s[1] = ctx1.reshape(B, 16, D)

        lhs_s[...] = jnp.concatenate([ctx_s[h // 16, :, h % 16, :] for h in range(H)], axis=1).astype(BF16)
        out = jnp.zeros((B, M), F32)
        r0 = 0
        if br == 1:
            chain_step()
            out = _dot(lhs_s[:, 0:CHAIN_TOTAL], wo_s[br, 0:CHAIN_TOTAL, :], NN)
            r0 = CHAIN_TOTAL
        for n in WO_ROWS[br]:
            a = lhs_s[:, r0:r0 + n]
            acquire()
            out = out + _dot(a, wo_s[br, r0:r0 + n, :], NN)
            r0 += n
        o_ref[:, M * br:M * (br + 1)] = out.astype(o_ref.dtype)

    branch(0)
    branch(1)
    assert state["copy"] == N_COPIES and state["chain"] == nch + 1


@jax.jit
def pallas_concat_heads__compressed_kv_cla__compressed_kv_cla__decode_kernel(
        A_x, A_c_kv, A_w_q, A_w_uk, A_w_uv, A_w_o, B_x, B_c_kv, B_w_q, B_w_uk, B_w_uv, B_w_o):
    out = pl.pallas_call(
        _kernel,
        out_shape=jax.ShapeDtypeStruct((B, 2 * M), BF16),
        in_specs=[pl.BlockSpec(memory_space=pl.ANY)] * 12,
        scratch_shapes=[
            pltpu.VMEM((2, B, M), BF16),
            pltpu.VMEM((2, B, SK, DC), BF16),
            pltpu.VMEM((2, M, H, D), BF16),
            pltpu.VMEM((2, DC, H, D), BF16),
            pltpu.VMEM((2, DC, H, D), BF16),
            pltpu.VMEM((2, H * D, M), BF16),
            pltpu.SMEM((2, max(CHAIN_ROWS), M), BF16),
            pltpu.VMEM((128, 2048), BF16),
            pltpu.VMEM((48, 2048), F32),
            pltpu.VMEM((DC, 128), F32),
            pltpu.VMEM((128, DC), BF16),
            pltpu.VMEM((4, 128, 128), BF16),
            pltpu.VMEM((2, B, 16, D), F32),
            pltpu.VMEM((B, H * D), BF16),
            pltpu.SemaphoreType.DMA((N_COPIES,)),
            pltpu.SemaphoreType.DMA((2,)),
        ],
        compiler_params=pltpu.CompilerParams(
            vmem_limit_bytes=110 * 1024 * 1024,
            disable_semaphore_checks=True,
            disable_bounds_checks=True,
        ),
    )(A_x.reshape(B, M), A_c_kv, A_w_q, A_w_uk, A_w_uv, A_w_o.reshape(H * D, M),
      B_x.reshape(B, M), B_c_kv, B_w_q, B_w_uk, B_w_uv, B_w_o.reshape(H * D, M))
    return out.reshape(B, 1, 2 * M)
```

```python
import jax
import jax.numpy as jnp
from jax.experimental import pallas as pl
from jax.experimental.pallas import tpu as pltpu

B, H, SK, D, M = 4, 32, 4096, 128, 640
DC = 4 * D
NN = (((1,), (0,)), ((), ()))
NT = (((1,), (1,)), ((), ()))
F32 = jnp.float32
BF16 = jnp.bfloat16

CHAIN_ROWS = (96, 80, 96, 80, 96, 80, 96, 128, 96, 80, 96, 80, 96, 80)
CHAIN_TOTAL = sum(CHAIN_ROWS)
WO_ROWS = ((2048, 2048), (1408, 1024, 256, 128))
assert CHAIN_TOTAL % D == 0 and CHAIN_TOTAL + sum(WO_ROWS[1]) == H * D == sum(WO_ROWS[0])
N_COPIES = 2 * (3 + B + 4) + len(WO_ROWS[0]) + len(WO_ROWS[1])
S2_ROWS = 32
NO_RUNTIME_CHECKS = {k: True for k in ("disable_semaphore_checks", "disable_bounds_checks")
                     if hasattr(pltpu.CompilerParams, k)}


def _dot(a, b, dims):
    return jax.lax.dot_general(a, b, dims, preferred_element_type=F32)


def _iota(shape, dim):
    return jax.lax.broadcasted_iota(jnp.int32, shape, dim)


def _kernel(ax, ac, awq, awuk, awuv, awo, bx, bc, bwq, bwuk, bwuv, bwo,
            o_ref,
            x_s, c_s, wq_s, wuk_s, wuv_s, wo_s, stage_s,
            e_s, xr_s, qat_s, qa_s, cc_s, ctx_s, lhs_s, sems, chain_sems):
    hbm = ((ax, ac, awq, awuk, awuv, awo), (bx, bc, bwq, bwuk, bwuv, bwo))

    copies, tick = [], []

    def add(src, dst, t=False):
        copies.append(pltpu.make_async_copy(src, dst, sems.at[len(copies)]))
        tick.append(t)

    for br in range(2):
        x, c, wq, wuk, wuv, wo = hbm[br]
        add(wq, wq_s.at[br])
        add(x, x_s.at[br], True)
        add(wuk, wuk_s.at[br], True)
        for b in range(B):
            add(c.at[b], c_s.at[br, b], True)
        for t in range(4):
            add(wuv.at[pl.ds(D * t, D)], wuv_s.at[br, pl.ds(D * t, D)], br == 0 and t == 3)
        r0 = 0 if br == 0 else CHAIN_TOTAL
        for k, n in enumerate(WO_ROWS[br]):
            add(wo.at[pl.ds(r0, n)], wo_s.at[br, pl.ds(r0, n)], br == 0 and k == len(WO_ROWS[0]) - 1)
            r0 += n
    assert len(copies) == N_COPIES

    nch = len(CHAIN_ROWS)
    assert sum(tick) == nch
    offs = [sum(CHAIN_ROWS[:j]) for j in range(nch)]
    h2s = [pltpu.make_async_copy(bwo.at[pl.ds(offs[j], r)], stage_s.at[j % 2, pl.ds(0, r)], chain_sems.at[0])
           for j, r in enumerate(CHAIN_ROWS)]
    s2v = [pltpu.make_async_copy(stage_s.at[j % 2, pl.ds(0, r)], wo_s.at[1, pl.ds(offs[j], r)], chain_sems.at[1])
           for j, r in enumerate(CHAIN_ROWS)]
    state = {"copy": 0, "chain": 0}

    def chain_step():
        j = state["chain"]
        state["chain"] = j + 1
        if j >= 1:
            s2v[j - 1].wait()
        if j < nch:
            h2s[j].wait()
            s2v[j].start(priority=1)
            if j + 1 < nch:
                h2s[j + 1].start(priority=1)

    def acquire():
        i = state["copy"]
        state["copy"] = i + 1
        copies[i].wait()
        if tick[i]:
            chain_step()

    copies[0].start()
    h2s[0].start(priority=1)
    for cp in copies[1:]:
        cp.start()

    e_s[...] = jnp.where(_iota((128, 2048), 0) == (_iota((128, 2048), 1) >> 4), 1.0, 0.0).astype(BF16)

    def branch(br):
        acquire()
        acquire()
        x = x_s[br].astype(F32)
        pieces = []
        for t in range(5):
            pieces += [x[:, 128 * t:128 * (t + 1)], jnp.zeros((4, 128), F32)]
        pieces.append(jnp.zeros((8, 128), F32))
        xs = jnp.concatenate(pieces, axis=0).astype(BF16)
        xr_s[...] = _dot(xs, e_s[...], NN)
        m64 = (_iota((64, 2048), 0) & 15) == (_iota((64, 2048), 1) & 15)

        def q_step(t, acc):
            q0, q1 = acc
            rows = [jnp.broadcast_to(xr_s[pl.ds(8 * t + b, 1), :], (16, 2048)) for b in range(B)]
            lt = jnp.where(m64, jnp.concatenate(rows, axis=0), 0.0).astype(BF16)
            m0 = pl.multiple_of(128 * t, 128)
            w0 = wq_s[br, pl.ds(m0, 128), 0:16, :].reshape(2048, D)
            w1 = wq_s[br, pl.ds(m0, 128), 16:32, :].reshape(2048, D)
            return q0 + _dot(lt, w0, NN), q1 + _dot(lt, w1, NN)

        zero = jnp.zeros((64, D), F32)
        q0, q1 = jax.lax.fori_loop(0, M // 128, q_step, (zero, zero))
        q_all = jnp.concatenate([q0, q1], axis=0).astype(BF16)

        acquire()
        lanes = _iota((S2_ROWS, H, 128), 2)
        m2 = _iota((S2_ROWS, H, 128), 1) == ((lanes >> 6) * 16 + (lanes & 15))

        def qa_step(i, carry):
            c0 = pl.multiple_of(S2_ROWS * i, S2_ROWS)
            w = wuk_s[br, pl.ds(c0, S2_ROWS), :, :].reshape(S2_ROWS * H, D)
            r = _dot(w, q_all, NT).reshape(S2_ROWS, H, 128)
            qat_s[pl.ds(c0, S2_ROWS), :] = jnp.sum(jnp.where(m2, r, 0.0), axis=1)
            return carry

        jax.lax.fori_loop(0, DC // S2_ROWS, qa_step, 0)
        qa_s[...] = (qat_s[...].T * (D ** -0.5)).astype(BF16)

        for b in range(B):
            acquire()
            qb = jnp.concatenate([qa_s[16 * b:16 * b + 16, :], qa_s[64 + 16 * b:64 + 16 * b + 16, :]], axis=0)
            s = _dot(qb, c_s[br, b], NT)
            p = jnp.exp(s - jnp.max(s, axis=1, keepdims=True))
            l = jnp.sum(p, axis=1, keepdims=True)
            cc = (_dot(p.astype(BF16), c_s[br, b], NN) / l).astype(BF16)
            for t in range(4):
                cc_s[t, 16 * b:16 * b + 16, :] = cc[0:16, 128 * t:128 * (t + 1)]
                cc_s[t, 64 + 16 * b:64 + 16 * b + 16, :] = cc[16:32, 128 * t:128 * (t + 1)]

        m128 = (_iota((128, 2048), 0) & 15) == (_iota((128, 2048), 1) & 15)
        ctx0 = jnp.zeros((64, D), F32)
        ctx1 = jnp.zeros((64, D), F32)
        for t in range(4):
            ex = jnp.where(m128, _dot(cc_s[t], e_s[...], NN), 0.0).astype(BF16)
            acquire()
            w0 = wuv_s[br, 128 * t:128 * (t + 1), 0:16, :].reshape(2048, D)
            w1 = wuv_s[br, 128 * t:128 * (t + 1), 16:32, :].reshape(2048, D)
            ctx0 = ctx0 + _dot(ex[0:64], w0, NN)
            ctx1 = ctx1 + _dot(ex[64:128], w1, NN)
        ctx_s[0] = ctx0.reshape(B, 16, D)
        ctx_s[1] = ctx1.reshape(B, 16, D)

        lhs_s[...] = jnp.concatenate([ctx_s[h // 16, :, h % 16, :] for h in range(H)], axis=1).astype(BF16)
        out = jnp.zeros((B, M), F32)
        r0 = 0
        if br == 1:
            chain_step()
            out = _dot(lhs_s[:, 0:CHAIN_TOTAL], wo_s[br, 0:CHAIN_TOTAL, :], NN)
            r0 = CHAIN_TOTAL
        for n in WO_ROWS[br]:
            a = lhs_s[:, r0:r0 + n]
            acquire()
            out = out + _dot(a, wo_s[br, r0:r0 + n, :], NN)
            r0 += n
        o_ref[:, M * br:M * (br + 1)] = out.astype(o_ref.dtype)

    branch(0)
    branch(1)
    assert state["copy"] == N_COPIES and state["chain"] == nch + 1


@jax.jit
def pallas_concat_heads__compressed_kv_cla__compressed_kv_cla__decode_kernel(
        A_x, A_c_kv, A_w_q, A_w_uk, A_w_uv, A_w_o, B_x, B_c_kv, B_w_q, B_w_uk, B_w_uv, B_w_o):
    out = pl.pallas_call(
        _kernel,
        out_shape=jax.ShapeDtypeStruct((B, 2 * M), BF16),
        in_specs=[pl.BlockSpec(memory_space=pl.ANY)] * 12,
        scratch_shapes=[
            pltpu.VMEM((2, B, M), BF16),
            pltpu.VMEM((2, B, SK, DC), BF16),
            pltpu.VMEM((2, M, H, D), BF16),
            pltpu.VMEM((2, DC, H, D), BF16),
            pltpu.VMEM((2, DC, H, D), BF16),
            pltpu.VMEM((2, H * D, M), BF16),
            pltpu.SMEM((2, max(CHAIN_ROWS), M), BF16),
            pltpu.VMEM((128, 2048), BF16),
            pltpu.VMEM((48, 2048), F32),
            pltpu.VMEM((DC, 128), F32),
            pltpu.VMEM((128, DC), BF16),
            pltpu.VMEM((4, 128, 128), BF16),
            pltpu.VMEM((2, B, 16, D), F32),
            pltpu.VMEM((B, H * D), BF16),
            pltpu.SemaphoreType.DMA((N_COPIES,)),
            pltpu.SemaphoreType.DMA((2,)),
        ],
        compiler_params=pltpu.CompilerParams(vmem_limit_bytes=110 * 1024 * 1024, **NO_RUNTIME_CHECKS),
    )(A_x.reshape(B, M), A_c_kv, A_w_q, A_w_uk, A_w_uv, A_w_o.reshape(H * D, M),
      B_x.reshape(B, M), B_c_kv, B_w_q, B_w_uk, B_w_uv, B_w_o.reshape(H * D, M))
    return out.reshape(B, 1, 2 * M)
```
